```python
import jax
import jax.numpy as jnp

def _softmax(x, axis=-1):
    return jax.nn.softmax(x, axis=axis)

def _gelu(x):
    return jax.nn.gelu(x, approximate=True)

def _silu(x):
    return jax.nn.silu(x)

def _sigmoid(x):
    return jax.nn.sigmoid(x)

def _layernorm(x, axis=-1, eps=1e-05):
    m = jnp.mean(x, axis=axis, keepdims=True)
    v = jnp.var(x, axis=axis, keepdims=True)
    return (x - m) / jnp.sqrt(v + eps)

def _scatter_add(tgt, idx, src, axis=0):
    return tgt.at[idx].add(src)

def _segment_sum(src, seg, n):
    return jax.ops.segment_sum(src, seg, n)

class _Rng:

    def __init__(self, key):
        self._k = key

    def _next(self):
        self._k, sub = jax.random.split(self._k)
        return sub

    def normal(self, shape):
        return jax.random.normal(self._next(), shape, dtype=jnp.bfloat16)

    def randint(self, lo, hi, shape):
        return jax.random.randint(self._next(), shape, lo, hi, dtype=jnp.int32)

    def uniform(self, shape, lo=0.0, hi=1.0):
        return jax.random.uniform(self._next(), shape, jnp.bfloat16, lo, hi)

    def permutation(self, n):
        return jax.random.permutation(self._next(), n)
kernel_name = 'adaLN_cond__softmax_full_mha__swiglu_ffn__prompt'

def _fwd_setup_inputs():
    _rng = _Rng(jax.random.key(int.from_bytes(__import__("os").urandom(4), "little")))
    _w = lambda a: (lambda t: t.astype(jnp.bfloat16) if jnp.issubdtype(t.dtype, jnp.floating) else t)(jnp.asarray(a))

    def _A_setup():
        B, S, D = (1, 2048, 448)
        return {'x': _w((lambda *s: _rng.normal(s) * 0.05)(B, S, D)), 'wqkv': _w((lambda *s: _rng.normal(s) * 0.05)(D, 3 * D)), 'wo': _w((lambda *s: _rng.normal(s) * 0.05)(D, D))}
    _A_in = _A_setup()

    def _B_setup():
        B, S, D, F = (1, 2048, 448, 1792)
        return {'x': _w((lambda *s: _rng.normal(s) * 0.05)(B, S, D)), 'w_gate': _w((lambda *s: _rng.normal(s) * 0.05)(D, F)), 'w_up': _w((lambda *s: _rng.normal(s) * 0.05)(D, F)), 'w_down': _w((lambda *s: _rng.normal(s) * 0.05)(F, D))}
    _B_in = _B_setup()
    return {'A_x': _A_in['x'], 'A_wqkv': _A_in['wqkv'], 'A_wo': _A_in['wo'], 'B_x': _B_in['x'], 'B_w_gate': _B_in['w_gate'], 'B_w_up': _B_in['w_up'], 'B_w_down': _B_in['w_down'], 'c': _w((lambda *s: _rng.normal(s) * 0.05)(1, 448)), 'w_mod': _w((lambda *s: _rng.normal(s) * 0.05)(448, 6 * 448) * 448 ** (-0.5))}

def _fwd_reference(A_x, A_wqkv, A_wo, B_x, B_w_gate, B_w_up, B_w_down, c, w_mod):

    def _A_ref(x, wqkv, wo):
        B, S, D = x.shape
        H = 16
        Dh = D // H
        qkv = (lambda x, *d: x.transpose(*d))((x @ wqkv).reshape(B, S, 3, H, Dh), 2, 0, 3, 1, 4)
        q, k, v = (qkv[0], qkv[1], qkv[2])
        scale = Dh ** (-0.5)
        scores = jnp.einsum('bhqd,bhkd->bhqk', q, k) * scale
        p = _softmax(scores, axis=-1)
        o = jnp.einsum('bhqk,bhkd->bhqd', p, v)
        return (lambda x, *d: x.transpose(*d))(o, 0, 2, 1, 3).reshape(B, S, D) @ wo

    def _B_ref(x, w_gate, w_up, w_down):
        g = _silu(x @ w_gate)
        u = x @ w_up
        return g * u @ w_down
    x = A_x
    mod = (_silu(c) @ w_mod).reshape(c.shape[0], 6, 1, -1)
    sa, ca, ga, sb, cb, gb = (mod[:, 0].copy(), mod[:, 1].copy(), mod[:, 2].copy(), mod[:, 3].copy(), mod[:, 4].copy(), mod[:, 5].copy())
    h = _layernorm(x, axis=-1) * (1 + ca) + sa
    x = x + ga * _A_ref(h, A_wqkv, A_wo)
    h = _layernorm(x, axis=-1) * (1 + cb) + sb
    x = x + gb * _B_ref(h, B_w_gate, B_w_up, B_w_down)
    return x

def setup_inputs():
    _inp = _fwd_setup_inputs()
    _gk = jax.random.fold_in(jax.random.key(int.from_bytes(__import__("os").urandom(4), "little")), 2 ** 31 - 1)
    _shapes = [[1, 2048, 448]]
    _dtypes = ['bfloat16']
    _gks = jax.random.split(_gk, len(_shapes))
    _gs = [jax.random.normal(k, s, dtype=jnp.dtype(d)) * 0.05 for k, s, d in zip(_gks, _shapes, _dtypes)]
    _inp['grad_out'] = _gs[0]
    return _inp

def reference(A_x, A_wqkv, A_wo, B_w_gate, B_w_up, B_w_down, c, w_mod, B_x, grad_out):
    _const = dict(B_x=B_x)

    def _f(*_d):
        return _fwd_reference(**{'A_x': _d[0], 'A_wqkv': _d[1], 'A_wo': _d[2], 'B_w_gate': _d[3], 'B_w_up': _d[4], 'B_w_down': _d[5], 'c': _d[6], 'w_mod': _d[7], **_const})
    _out, _vjp = jax.vjp(_f, A_x, A_wqkv, A_wo, B_w_gate, B_w_up, B_w_down, c, w_mod)
    _grads = _vjp(grad_out)
    _out0 = jnp.asarray(_out)
    return (_out0, *[jnp.asarray(_g) for _g in _grads])
```

```python
import jax
import jax.numpy as jnp
from jax.experimental import pallas as pl
from jax.experimental.pallas import tpu as pltpu

F32 = jnp.float32
BF16 = jnp.bfloat16

T, D, H, DH, F = 2048, 448, 16, 28, 1792
DP = 32
HP = H * DP
NTT = T // 128
BQ = 256
NQ = BQ // 128
NB = T // BQ
FC = 128
NF = F // FC
KG = 4 // NQ
NG = NTT // KG
UF, LAGF = 2, 3
UB, LAGB = 2, 2
EPS = 1e-5
SCALE = DH ** -0.5
LOG2E = 1.4426950408889634
LN2 = 0.6931471805599453
SAFE_BOUND = 40.0

_NT = (((1,), (1,)), ((), ()))


def _dot(a, b):
    return jnp.dot(a, b, preferred_element_type=F32)


def _dot_nt(a, b):
    return jax.lax.dot_general(a, b, _NT, preferred_element_type=F32)


def _split3(v):
    hi = v.astype(BF16).astype(F32)
    r = v - hi
    mid = r.astype(BF16).astype(F32)
    lo = (r - mid).astype(BF16).astype(F32)
    return hi, mid, lo


def _unpad_windows(n_out):
    res = []
    for s in range(0, n_out, 128):
        w = min(128, n_out - s)
        p0 = DP * (s // DH) + s % DH
        p1 = DP * ((s + w - 1) // DH) + (s + w - 1) % DH
        a = (p0 // 128) * 128
        b = (p1 // 128 + 1) * 128
        res.append((s, w, a, b - a))
    return res


def _kernel(x_hbm, wqkv_hbm, wo_hbm, wg_hbm, wu_hbm, wd_hbm, wmod_hbm, dy_hbm, c_ref,
            out_hbm, dx_hbm, dwqkv_hbm, dwo_hbm, dwg_hbm, dwu_hbm, dwd_hbm, dc_ref, dwmod_hbm,
            x_in, dy_in, wqkv_in, wo_in, wg_in, wu_in, wd_in, wmod_in,
            wqkvT, wqkvP, woT, woP, wgT, wuT, wdN, tmp_pad,
            modc, dmodp,
            xh1, st1, h1T, qT, kT, vT, k_tm, v_tm, dkT, dvT, dqkvT, dx1T, nrm,
            wq, wdo, p_s, ds_s, ot, otb, rl_s, x1, attn, xh2, st2, h2, dffn,
            ffn, dh2, actA, dguA, actB, dguB, dattn, dob,
            dwg_acc, dwu_acc, dwd_acc, dwo_acc, dwqkv_pad,
            out_st, dx_st, dwg_st, dwu_st, dwd_st, dwo_st, dwqkv_st, dwmod_st,
            flag, sems):

    def cp(src, dst, i):
        return pltpu.make_async_copy(src, dst, sems.at[i])

    cp_x = cp(x_hbm, x_in, 0)
    cp_wmod = cp(wmod_hbm, wmod_in, 1)
    cp_wqkv = cp(wqkv_hbm, wqkv_in, 2)
    cp_wo = cp(wo_hbm, wo_in, 3)
    cp_dy = cp(dy_hbm, dy_in, 4)
    cp_wg = cp(wg_hbm, wg_in, 5)
    cp_wu = cp(wu_hbm, wu_in, 6)
    cp_wd = cp(wd_hbm, wd_in, 7)
    cp_x.start()
    cp_wmod.start()
    cp_wqkv.start()
    cp_wo.start()
    cp_wg.start()
    cp_wu.start()
    cp_wd.start()
    cp_dy.start()

    for ref in (dwg_acc, dwu_acc, dwd_acc, dwo_acc, dkT, dvT, wq, wdo, dmodp):
        ref[...] = jnp.zeros(ref.shape, ref.dtype)
    nrm[...] = jnp.zeros(nrm.shape, F32)

    cp_x.wait()

    def ln1_body(t, carry):
        r0 = pl.multiple_of(t * 128, 128)
        xf = x_in[:, pl.ds(r0, 128)].astype(F32)
        mu = jnp.mean(xf, axis=0, keepdims=True)
        xc = xf - mu
        var = jnp.mean(xc * xc, axis=0, keepdims=True)
        rs = jax.lax.rsqrt(var + EPS)
        xh1[t] = xc * rs
        st1[t] = jnp.broadcast_to(rs, (8, 128))
        return carry

    jax.lax.fori_loop(0, NTT, ln1_body, 0)

    cp_wmod.wait()
    c = c_ref[...].astype(F32)
    sig_c = 1.0 / (1.0 + jnp.exp(-c))
    sc = c * sig_c
    row16 = jax.lax.broadcasted_iota(jnp.int32, (16, D), 0)
    hi, mid, lo = _split3(sc)
    sc3 = jnp.where(row16 == 0, hi, jnp.where(row16 == 1, mid, jnp.where(row16 == 2, lo, 0.0)))
    mod3 = _dot(sc3.astype(BF16), wmod_in[...])
    mod = mod3[0:1] + mod3[1:2] + mod3[2:3]
    for i in range(6 * D // 128):
        modc[i * 128:(i + 1) * 128, :] = jnp.broadcast_to(mod[:, i * 128:(i + 1) * 128], (128, 128)).T

    def mcol(i):
        return modc[i * D:(i + 1) * D, :]

    SA, CA, GA, SB, CB, GB = range(6)

    cp_wqkv.wait()
    wqkvT[...] = jnp.zeros(wqkvT.shape, BF16)
    for i in range(3 * D // 128 + 1):
        w = min(128, 3 * D - i * 128)
        tmp_pad[i * 128:i * 128 + w, :] = wqkv_in[:, i * 128:i * 128 + w].T
    for h in range(3 * H):
        wqkvT[DP * h:DP * h + DH, :] = tmp_pad[DH * h:DH * h + DH, :]
    for i in range(3 * HP // 128):
        wqkvP[:, i * 128:(i + 1) * 128] = wqkvT[i * 128:(i + 1) * 128, :].T

    cp_wo.wait()
    woP[...] = jnp.zeros(woP.shape, BF16)
    for h in range(H):
        woP[DP * h:DP * h + DH, :] = wo_in[DH * h:DH * h + DH, :]
    for i in range(HP // 128):
        woT[:, i * 128:(i + 1) * 128] = woP[i * 128:(i + 1) * 128, :].T

    QC = 256
    rowq = jax.lax.broadcasted_iota(jnp.int32, (QC, 128), 0) % DP
    is_one = jnp.logical_and(rowq >= DH, rowq < DH + 3)

    def qkv_body(t, carry):
        r0 = pl.multiple_of(t * 128, 128)
        h1 = (xh1[t] * (1.0 + mcol(CA)) + mcol(SA)).astype(BF16)
        h1T[t] = h1
        for ci in range(3 * HP // QC):
            r = _dot(wqkvT[ci * QC:(ci + 1) * QC, :], h1)
            part, sub = divmod(ci, HP // QC)
            rows = slice(sub * QC, (sub + 1) * QC)
            if part == 0:
                r = r * (SCALE * LOG2E)
                qT[t, rows, :] = r.astype(BF16)
                n2 = jnp.sum((r * r).reshape(QC // DP, DP, 128), axis=1)
                nrm[sub] = jnp.maximum(nrm[sub], n2)
            else:
                if part == 1:
                    n2 = jnp.sum((r * r).reshape(QC // DP, DP, 128), axis=1)
                    nrm[2 + sub] = jnp.maximum(nrm[2 + sub], n2)
                rb = jnp.where(is_one, 1.0, r).astype(BF16)
                dst_t, dst_tm = (kT, k_tm) if part == 1 else (vT, v_tm)
                dst_t[t, rows, :] = rb
                for gi in range(QC // 128):
                    dst_tm[sub * (QC // 128) + gi, pl.ds(r0, 128), :] = rb[gi * 128:(gi + 1) * 128, :].T
        return carry

    jax.lax.fori_loop(0, NTT, qkv_body, 0)

    qmax = jnp.max(nrm[0:2], axis=2, keepdims=True)
    kmax = jnp.max(nrm[2:4], axis=2, keepdims=True)
    bound2 = jnp.max(qmax * kmax)
    flag[0] = jnp.where(bound2 <= SAFE_BOUND * SAFE_BOUND, 0, 1).astype(jnp.int32)

    cp_wg.wait()
    cp_wu.wait()
    cp_wd.wait()

    def wt_body(f, carry):
        o = pl.multiple_of(f * 128, 128)
        wgT[pl.ds(o, 128), :] = wg_in[:, pl.ds(o, 128)].T
        wuT[pl.ds(o, 128), :] = wu_in[:, pl.ds(o, 128)].T
        wdN[pl.ds(o, 128), :] = wd_in[:, pl.ds(o, 128)].T
        return carry

    jax.lax.fori_loop(0, F // 128, wt_body, 0)
    cp_dy.wait()

    row16l = jax.lax.broadcasted_iota(jnp.int32, (16, 128), 0)

    def put3(base16, v):
        hi, mid, lo = _split3(v)
        return jnp.where(row16l == 12, -hi,
                         jnp.where(row16l == 13, -mid, jnp.where(row16l == 14, -lo, base16)))

    def block_body(b, carry):
        tq = [b * NQ + j for j in range(NQ)]
        lanes = [slice(j * 128, (j + 1) * 128) for j in range(NQ)]

        def wq_body(h, c2):
            src = pl.multiple_of(h * DP, DP)
            dst = pl.multiple_of((h % 4) * DP, DP)
            for j in range(NQ):
                wq[h, j, pl.ds(dst, DP), :] = qT[tq[j], pl.ds(src, DP), :]
            return c2

        jax.lax.fori_loop(0, H, wq_body, 0)

        @pl.when(flag[0] != 0)
        def _():
            def max_body(h, c2):
                g = h // 4
                dst = pl.multiple_of((h % 4) * DP + 16, 16)
                for j in range(NQ):
                    m = None
                    for t in range(NTT):
                        s = _dot(k_tm[g, t * 128:(t + 1) * 128, :], wq[h, j])
                        m = s if m is None else jnp.maximum(m, s)
                    m = jnp.max(m, axis=0, keepdims=True)
                    old = wq[h, j, pl.ds(dst, 16), :].astype(F32)
                    wq[h, j, pl.ds(dst, 16), :] = put3(old, m).astype(BF16)
                return c2

            jax.lax.fori_loop(0, H, max_body, 0)

        def s_group(h, gi):
            g = h // 4
            for t in range(gi * KG, (gi + 1) * KG):
                kc = k_tm[g, t * 128:(t + 1) * 128, :]
                for j in range(NQ):
                    s = _dot(kc, wq[h, j])
                    p_s[h, j, t * 128:(t + 1) * 128, :] = jnp.exp2(s).astype(BF16)

        def pv_group(h, gi, acc):
            hr = pl.multiple_of(h * DP, DP)
            for t in range(gi * KG, (gi + 1) * KG):
                for j in range(NQ):
                    r = _dot(vT[t, pl.ds(hr, DP), :], p_s[h, j, t * 128:(t + 1) * 128, :])
                    acc[j] = r if acc[j] is None else acc[j] + r

        def fwd_body(i, c2):
            seq = [(i * UF + u, u, gi) for u in range(UF) for gi in range(NG)]
            accs = {}
            for n in range(len(seq) + LAGF):
                if n < len(seq):
                    s_group(seq[n][0], seq[n][2])
                if n >= LAGF:
                    h, u, gi = seq[n - LAGF]
                    if gi == 0:
                        accs[u] = [None] * NQ
                    pv_group(h, gi, accs[u])
                    if gi == NG - 1:
                        hr = pl.multiple_of(h * DP, DP)
                        for j in range(NQ):
                            ot[pl.ds(hr, DP), lanes[j]] = accs[u][j]
            return c2

        jax.lax.fori_loop(0, H // UF, fwd_body, 0)

        for j in range(NQ):
            o3 = ot[:, lanes[j]].reshape(H, DP, 128)
            rl = 1.0 / o3[:, DH:DH + 1, :]
            o3 = (o3 * rl).reshape(HP, 128)
            ot[:, lanes[j]] = o3
            otb[:, lanes[j]] = o3.astype(BF16)
            rl_s[j] = rl

        at = _dot(woT[...], otb[...])
        attn[...] = at
        for j in range(NQ):
            r0 = pl.multiple_of(tq[j] * 128, 128)
            x1j = x_in[:, pl.ds(r0, 128)].astype(F32) + mcol(GA) * attn[:, lanes[j]]
            x1[:, lanes[j]] = x1j
            mu = jnp.mean(x1j, axis=0, keepdims=True)
            xc = x1j - mu
            var = jnp.mean(xc * xc, axis=0, keepdims=True)
            rs = jax.lax.rsqrt(var + EPS)
            xh = xc * rs
            xh2[:, lanes[j]] = xh
            st2[j] = jnp.broadcast_to(rs, (8, 128))
            h2[:, lanes[j]] = (xh * (1.0 + mcol(CB)) + mcol(SB)).astype(BF16)
            dyt = dy_in[:, pl.ds(r0, 128)].astype(F32)
            dffn[:, lanes[j]] = (dyt * mcol(GB)).astype(BF16)
        ffn[...] = jnp.zeros(ffn.shape, F32)
        dh2[...] = jnp.zeros(dh2.shape, F32)

        def ffn_a(f, act_buf, dgu_buf):
            o = pl.multiple_of(f * FC, FC)
            g = _dot(wgT[pl.ds(o, FC), :], h2[...])
            u = _dot(wuT[pl.ds(o, FC), :], h2[...])
            da = _dot(wdN[pl.ds(o, FC), :], dffn[...])
            sg = 0.5 * jnp.tanh(0.5 * g) + 0.5
            si = g * sg
            act_buf[...] = (si * u).astype(BF16)
            dgu_buf[0:FC, :] = (da * u * (sg + si * (1.0 - sg))).astype(BF16)
            dgu_buf[FC:2 * FC, :] = (da * si).astype(BF16)

        def ffn_b(f, act_buf, dgu_buf):
            o = pl.multiple_of(f * FC, FC)
            cols = pl.ds(o, FC)
            ffn[...] += _dot(wd_in[:, cols], act_buf[...])
            dh2[...] += _dot(wg_in[:, cols], dgu_buf[0:FC, :]) + _dot(wu_in[:, cols], dgu_buf[FC:2 * FC, :])
            dgu = _dot_nt(h2[...], dgu_buf[...])
            dwg_acc[:, cols] += dgu[:, 0:FC]
            dwu_acc[:, cols] += dgu[:, FC:2 * FC]
            dwd_acc[:, cols] += _dot_nt(dffn[...], act_buf[...])

        ffn_a(0, actA, dguA)

        def ffn_body(i, c2):
            f = 2 * i
            ffn_a(f + 1, actB, dguB)
            ffn_b(f, actA, dguA)
            ffn_a(jnp.minimum(f + 2, NF - 1), actA, dguA)
            ffn_b(f + 1, actB, dguB)
            return c2

        jax.lax.fori_loop(0, NF // 2, ffn_body, 0)

        out_cp = pltpu.make_async_copy(out_st, out_hbm.at[:, pl.ds(pl.multiple_of(b * BQ, BQ), BQ)], sems.at[8])

        @pl.when(b > 0)
        def _():
            out_cp.wait()

        for j in range(NQ):
            fj = ffn[:, lanes[j]]
            dyt = dy_in[:, pl.ds(pl.multiple_of(tq[j] * 128, 128), 128)].astype(F32)
            o = x1[:, lanes[j]] + mcol(GB) * fj
            out_st[:, lanes[j]] = o.astype(BF16)
            dmodp[GB * D:(GB + 1) * D, :] += dyt * fj
            dh = dh2[:, lanes[j]]
            xh = xh2[:, lanes[j]]
            dmodp[SB * D:(SB + 1) * D, :] += dh
            dmodp[CB * D:(CB + 1) * D, :] += dh * xh
            dxh = dh * (1.0 + mcol(CB))
            m1 = jnp.mean(dxh, axis=0, keepdims=True)
            m2 = jnp.mean(dxh * xh, axis=0, keepdims=True)
            dx1 = dyt + st2[j, 0:1, :] * (dxh - m1 - xh * m2)
            dx1T[tq[j]] = dx1
            dmodp[GA * D:(GA + 1) * D, :] += dx1 * attn[:, lanes[j]]
            dattn[:, lanes[j]] = (dx1 * mcol(GA)).astype(BF16)
        out_cp.start()

        dwo_acc[...] += _dot_nt(otb[...], dattn[...])
        do_all = _dot(woP[...], dattn[...])
        row32 = jax.lax.broadcasted_iota(jnp.int32, (H, DP, 128), 1)
        for j in range(NQ):
            do3 = do_all[:, lanes[j]].reshape(H, DP, 128)
            o3 = ot[:, lanes[j]].reshape(H, DP, 128)
            rl = rl_s[j]
            delta = jnp.sum(do3 * o3, axis=1, keepdims=True) * rl
            hi, mid, lo = _split3(delta)
            do3 = jnp.where(row32 == DH, -hi,
                            jnp.where(row32 == DH + 1, -mid, jnp.where(row32 == DH + 2, -lo, do3 * rl)))
            dob[j] = do3.reshape(HP, 128).astype(BF16)

        def wdo_body(h, c2):
            src = pl.multiple_of(h * DP, DP)
            dst = pl.multiple_of((h % 4) * DP, DP)
            for j in range(NQ):
                wdo[h, j, pl.ds(dst, DP), :] = dob[j, pl.ds(src, DP), :]
            return c2

        jax.lax.fori_loop(0, H, wdo_body, 0)

        def dp_group(h, u, gi):
            g = h // 4
            for t in range(gi * KG, (gi + 1) * KG):
                vc = v_tm[g, t * 128:(t + 1) * 128, :]
                for j in range(NQ):
                    dp = _dot(vc, wdo[h, j])
                    p = p_s[h, j, t * 128:(t + 1) * 128, :].astype(F32)
                    ds_s[u % 2, j, t * 128:(t + 1) * 128, :] = (p * dp).astype(BF16)

        def g_group(h, u, gi, acc):
            hr = pl.multiple_of(h * DP, DP)
            ts = list(range(gi * KG, (gi + 1) * KG))
            dk, dv = {}, {}
            for t in ts:
                for j in range(NQ):
                    r = _dot_nt(qT[tq[j], pl.ds(hr, DP), :], ds_s[u % 2, j, t * 128:(t + 1) * 128, :])
                    dk[t] = r if t not in dk else dk[t] + r
            for t in ts:
                for j in range(NQ):
                    r = _dot_nt(dob[j, pl.ds(hr, DP), :], p_s[h, j, t * 128:(t + 1) * 128, :])
                    dv[t] = r if t not in dv else dv[t] + r
            for t in ts:
                for j in range(NQ):
                    r = _dot(kT[t, pl.ds(hr, DP), :], ds_s[u % 2, j, t * 128:(t + 1) * 128, :])
                    acc[j] = r if acc[j] is None else acc[j] + r
            for t in ts:
                dkT[t, pl.ds(hr, DP), :] += dk[t]
                dvT[t, pl.ds(hr, DP), :] += dv[t]

        def bwd_body(i, c2):
            seq = [(i * UB + u, u, gi) for u in range(UB) for gi in range(NG)]
            accs = {}
            for n in range(len(seq) + LAGB):
                if n < len(seq):
                    dp_group(*seq[n])
                if n >= LAGB:
                    h, u, gi = seq[n - LAGB]
                    if gi == 0:
                        accs[u] = [None] * NQ
                    g_group(h, u, gi, accs[u])
                    if gi == NG - 1:
                        hr = pl.multiple_of(h * DP, DP)
                        for j in range(NQ):
                            dqkvT[tq[j], pl.ds(hr, DP), :] = (accs[u][j] * SCALE).astype(BF16)
            return c2

        jax.lax.fori_loop(0, H // UB, bwd_body, 0)
        return carry

    jax.lax.fori_loop(0, NB, block_body, 0)
    pltpu.make_async_copy(out_st, out_hbm.at[:, pl.ds((NB - 1) * BQ, BQ)], sems.at[8]).wait()

    dwg_st[...] = dwg_acc[...].astype(BF16)
    cp_dwg = cp(dwg_st, dwg_hbm, 9)
    cp_dwg.start()
    dwu_st[...] = dwu_acc[...].astype(BF16)
    cp_dwu = cp(dwu_st, dwu_hbm, 10)
    cp_dwu.start()
    dwd_st[...] = dwd_acc[...].astype(BF16)
    cp_dwd = cp(dwd_st, dwd_hbm, 11)
    cp_dwd.start()
    for h in range(H):
        dwo_st[DH * h:DH * h + DH, :] = dwo_acc[DP * h:DP * h + DH, :].astype(BF16)
    cp_dwo = cp(dwo_st, dwo_hbm, 12)
    cp_dwo.start()

    def dkv_body(t, carry):
        dqkvT[t, HP:2 * HP, :] = (dkT[t] * LN2).astype(BF16)
        dqkvT[t, 2 * HP:3 * HP, :] = dvT[t].astype(BF16)
        return carry

    jax.lax.fori_loop(0, NTT, dkv_body, 0)

    def dwqkv_body(n, carry):
        o = pl.multiple_of(n * 128, 128)
        acc = None
        for t in range(NTT):
            r = _dot_nt(h1T[t], dqkvT[t, pl.ds(o, 128), :])
            acc = r if acc is None else acc + r
        dwqkv_pad[:, pl.ds(o, 128)] = acc.astype(BF16)
        return carry

    jax.lax.fori_loop(0, 3 * HP // 128, dwqkv_body, 0)

    for (s, w, a, ww) in _unpad_windows(3 * D):
        pi = a + jax.lax.broadcasted_iota(jnp.int32, (ww, 128), 0)
        ui = s + jax.lax.broadcasted_iota(jnp.int32, (ww, 128), 1)
        hq = jnp.floor((ui.astype(F32) + 0.5) * (1.0 / DH)).astype(jnp.int32)
        e = jnp.where(pi == ui + (DP - DH) * hq, 1.0, 0.0).astype(BF16)
        r = _dot(dwqkv_pad[:, a:a + ww], e)
        dwqkv_st[:, s:s + w] = r[:, 0:w].astype(BF16)
    cp_dwqkv = cp(dwqkv_st, dwqkv_hbm, 13)
    cp_dwqkv.start()

    def dx_body(t, carry):
        dh = _dot(wqkvP[...], dqkvT[t])
        xh = xh1[t]
        dmodp[SA * D:(SA + 1) * D, :] += dh
        dmodp[CA * D:(CA + 1) * D, :] += dh * xh
        dxh = dh * (1.0 + mcol(CA))
        m1 = jnp.mean(dxh, axis=0, keepdims=True)
        m2 = jnp.mean(dxh * xh, axis=0, keepdims=True)
        dx = dx1T[t] + st1[t, 0:1, :] * (dxh - m1 - xh * m2)
        r0 = pl.multiple_of(t * 128, 128)
        dx_st[:, pl.ds(r0, 128)] = dx.astype(BF16)
        return carry

    jax.lax.fori_loop(0, NTT, dx_body, 0)
    cp_dx = cp(dx_st, dx_hbm, 14)
    cp_dx.start()

    parts = []
    for i in range(6 * D // 128):
        parts.append(jnp.sum(dmodp[i * 128:(i + 1) * 128, :].T, axis=0, keepdims=True))
    dmod = jnp.concatenate(parts, axis=1)
    row16m = jax.lax.broadcasted_iota(jnp.int32, (16, 6 * D), 0)
    hi, mid, lo = _split3(dmod)
    dm3 = jnp.where(row16m == 0, hi, jnp.where(row16m == 1, mid, jnp.where(row16m == 2, lo, 0.0)))
    dsc3 = _dot_nt(dm3.astype(BF16), wmod_in[...])
    dsc = dsc3[0:1] + dsc3[1:2] + dsc3[2:3]
    dc_ref[...] = (dsc * (sig_c * (1.0 + c * (1.0 - sig_c)))).astype(BF16)

    sccol = jnp.broadcast_to(sc, (128, D)).T
    for i in range(6 * D // 128):
        dwmod_st[:, i * 128:(i + 1) * 128] = (sccol * dmod[:, i * 128:(i + 1) * 128]).astype(BF16)
    cp_dwmod = cp(dwmod_st, dwmod_hbm, 15)
    cp_dwmod.start()

    for d in (cp_dwg, cp_dwu, cp_dwd, cp_dwo, cp_dwqkv, cp_dx, cp_dwmod):
        d.wait()


def _scratch():
    v = pltpu.VMEM
    return [
        v((D, T), BF16), v((D, T), BF16), v((D, 3 * D), BF16), v((D, D), BF16),
        v((D, F), BF16), v((D, F), BF16), v((D, F), BF16), v((D, 6 * D), BF16),
        v((3 * HP, D), BF16), v((D, 3 * HP), BF16), v((D, HP), BF16), v((HP, D), BF16),
        v((F, D), BF16), v((F, D), BF16), v((F, D), BF16), v((3 * D, D), BF16),
        v((6 * D, 128), F32), v((6 * D, 128), F32),
        v((NTT, D, 128), F32), v((NTT, 8, 128), F32), v((NTT, D, 128), BF16),
        v((NTT, HP, 128), BF16), v((NTT, HP, 128), BF16), v((NTT, HP, 128), BF16),
        v((4, T, 128), BF16), v((4, T, 128), BF16),
        v((NTT, HP, 128), F32), v((NTT, HP, 128), F32), v((NTT, 3 * HP, 128), BF16),
        v((NTT, D, 128), F32), v((4, 8, 128), F32),
        v((H, NQ, 128, 128), BF16), v((H, NQ, 128, 128), BF16),
        v((H, NQ, T, 128), BF16), v((2, NQ, T, 128), BF16),
        v((HP, BQ), F32), v((HP, BQ), BF16), v((NQ, H, 1, 128), F32),
        v((D, BQ), F32), v((D, BQ), F32), v((D, BQ), F32), v((NQ, 8, 128), F32),
        v((D, BQ), BF16), v((D, BQ), BF16),
        v((D, BQ), F32), v((D, BQ), F32),
        v((FC, BQ), BF16), v((2 * FC, BQ), BF16), v((FC, BQ), BF16), v((2 * FC, BQ), BF16),
        v((D, BQ), BF16), v((NQ, HP, 128), BF16),
        v((D, F), F32), v((D, F), F32), v((D, F), F32), v((HP, D), F32), v((D, 3 * HP), BF16),
        v((D, BQ), BF16), v((D, T), BF16), v((D, F), BF16), v((D, F), BF16), v((D, F), BF16),
        v((D, D), BF16), v((D, 3 * D), BF16), v((D, 6 * D), BF16),
        pltpu.SMEM((1,), jnp.int32),
        pltpu.SemaphoreType.DMA((16,)),
    ]


@jax.jit
def pallas_adaLN_cond__softmax_full_mha__swiglu_ffn__prompt_kernel(
    A_x: jax.Array,
    A_wqkv: jax.Array,
    A_wo: jax.Array,
    B_x: jax.Array,
    B_w_gate: jax.Array,
    B_w_up: jax.Array,
    B_w_down: jax.Array,
    c: jax.Array,
    w_mod: jax.Array,
    grad_out: jax.Array,
):
    del B_x
    sds = jax.ShapeDtypeStruct
    hbm = pl.BlockSpec(memory_space=pl.ANY)
    vmem = pl.BlockSpec(memory_space=pltpu.VMEM)
    outs = pl.pallas_call(
        _kernel,
        out_shape=(
            sds((D, T), BF16), sds((D, T), BF16), sds((D, 3 * D), BF16), sds((D, D), BF16),
            sds((D, F), BF16), sds((D, F), BF16), sds((D, F), BF16), sds((1, D), BF16),
            sds((D, 6 * D), BF16),
        ),
        in_specs=[hbm] * 8 + [vmem],
        out_specs=(hbm,) * 7 + (vmem, hbm),
        scratch_shapes=_scratch(),
        compiler_params=pltpu.CompilerParams(vmem_limit_bytes=120 * 1024 * 1024),
        name="adaln_block_fwd_bwd",
    )(A_x.reshape(T, D).T, A_wqkv, A_wo, B_w_gate, B_w_up, B_w_down.T, w_mod,
      grad_out.reshape(T, D).T, c)
    out, dx, dwqkv, dwo, dwg, dwu, dwd, dc, dwmod = outs
    return (out.T.reshape(1, T, D), dx.T.reshape(1, T, D), dwqkv, dwo, dwg, dwu, dwd.T, dc, dwmod)
```

```python
import jax
import jax.numpy as jnp
from jax.experimental import pallas as pl
from jax.experimental.pallas import tpu as pltpu

F32 = jnp.float32
BF16 = jnp.bfloat16

T, D, H, DH, F = 2048, 448, 16, 28, 1792
DP = 32
HP = H * DP
NTT = T // 128
BQ = 256
NQ = BQ // 128
NB = T // BQ
FC = 128
NF = F // FC
KG = 4 // NQ
NG = NTT // KG
HL = 8
NDA = H // HL + 3
LAGF = 7
LAGB = 2
NWC = -(-3 * D // 128)
EPS = 1e-5
SCALE = DH ** -0.5
LOG2E = 1.4426950408889634
LN2 = 0.6931471805599453
SAFE_BOUND = 40.0

_NT = (((1,), (1,)), ((), ()))


def _dot(a, b):
    return jnp.dot(a, b, preferred_element_type=F32)


def _dot_nt(a, b):
    return jax.lax.dot_general(a, b, _NT, preferred_element_type=F32)


def _split3(v):
    hi = v.astype(BF16).astype(F32)
    r = v - hi
    mid = r.astype(BF16).astype(F32)
    lo = (r - mid).astype(BF16).astype(F32)
    return hi, mid, lo


def _zero_after(v):
    return jnp.where(v != v, v, 0.0)


def _after(lhs, z):
    top = (lhs[0:16, :].astype(F32) + z).astype(BF16)
    return jnp.concatenate([top, lhs[16:, :]], axis=0)


def _interleave(main, side, first=1):
    slots = len(main) - first
    done = 0
    for i, job in enumerate(main):
        job()
        if i + 1 >= first:
            want = min(len(side), -(-(i + 2 - first) * len(side) // slots))
            while done < want:
                side[done]()
                done += 1


def _layernorm_stages(load, finish, first_load=None):
    st = {}

    def s1():
        x = load() if first_load is None else first_load()
        st["mu"] = jnp.mean(x, axis=0, keepdims=True)

    def s2():
        xc = load() - st["mu"]
        st["rs"] = jax.lax.rsqrt(jnp.mean(xc * xc, axis=0, keepdims=True) + EPS)

    def s3():
        finish((load() - st["mu"]) * st["rs"], st["rs"])

    return [s1, s2, s3]


def _kernel(x_hbm, wqkv_hbm, wo_hbm, wg_hbm, wu_hbm, wd_hbm, wmod_hbm, dy_hbm, c_ref,
            out_hbm, dx_hbm, dwqkv_hbm, dwo_hbm, dwg_hbm, dwu_hbm, dwd_hbm, dc_ref, dwmod_hbm,
            x_in, dy_in, wqkv_in, wo_in, wg_in, wu_in, wd_in, wmod_in,
            wqkvT, woT, woP, wgT, wuT, wdN, tmp_pad, s112, s128, s128u,
            modc, dmodp,
            xh1, st1, h1T, qT, kT, vT, k_tm, v_tm, dqT, dkT, dvT, dqkvU, cv_s, dx1T, nrm,
            wq, wdo, p_s, ds_s, ot, otb, rl_s, x1, attn, xh2, st2, h2, dffn,
            ffn, dh2, da_s, act_s, dgu_s, dattn, do_s, dob, dh_s,
            dwg_acc, dwu_acc, dwd_acc, dwo_acc,
            out_st, dx_st, dwg_st, dwu_st, dwd_st, dwo_st, dwqkv_st, dwqkv_last, dwmod_st,
            flag, sems):

    def cp(src, dst, i):
        return pltpu.make_async_copy(src, dst, sems.at[i])

    TA = 9
    XA = (TA + 1) * 128
    MA = 2 * D
    cp_wqkv = cp(wqkv_hbm, wqkv_in, 0)
    cp_wmod_a = cp(wmod_hbm.at[:, 0:MA], wmod_in.at[:, 0:MA], 1)
    cp_x_0 = cp(x_hbm.at[:, 0:128], x_in.at[:, 0:128], 12)
    cp_x_a = cp(x_hbm.at[:, 128:XA], x_in.at[:, 128:XA], 2)
    cp_x_b = cp(x_hbm.at[:, XA:T], x_in.at[:, XA:T], 3)
    cp_wmod_b = cp(wmod_hbm.at[:, MA:6 * D], wmod_in.at[:, MA:6 * D], 4)
    cp_wo = cp(wo_hbm, wo_in, 5)
    cp_wg = cp(wg_hbm, wg_in, 6)
    cp_wu = cp(wu_hbm, wu_in, 7)
    cp_wd = cp(wd_hbm, wd_in, 8)
    cp_dy = cp(dy_hbm, dy_in, 9)
    cp_wqkv.start()

    tile = [slice(t * 128, (t + 1) * 128) for t in range(6 * D // 128)]
    hrows = [slice(h * DP, (h + 1) * DP) for h in range(H)]

    def dtile(i):
        return pl.ds(pl.multiple_of(i * 128, 128), 128)

    def loop(n, fn, start=0):
        def body(i, carry):
            fn(i)
            return carry
        jax.lax.fori_loop(start, n, body, 0)

    def zero_head(h):
        wq[h] = jnp.zeros(wq.shape[1:], BF16)
        wdo[h] = jnp.zeros(wdo.shape[1:], BF16)

    loop(H, zero_head)

    def zero_dmod(i):
        dmodp[dtile(i), :] = jnp.zeros((128, 128), F32)

    loop(6 * D // 128, zero_dmod)
    nrm[...] = jnp.zeros(nrm.shape, F32)
    s128[...] = jnp.zeros(s128.shape, BF16)
    cp_x_0.start()
    cp_wmod_a.start()
    cp_x_a.start()

    GD = 4 * DH
    halves = [slice(0, D // 2), slice(D // 2, D)]

    def pad_stages(src, g, dst, k=0):
        def s1():
            s112[k] = src[pl.ds(pl.multiple_of(g * GD, 16), GD), :]

        def s2():
            for hh in range(4):
                s128[k, DP * hh:DP * hh + DH, :] = s112[k, DH * hh:DH * hh + DH, :]
            dst[dtile(g), :] = s128[k]

        return [s1, s2]

    cp_wqkv.wait()
    for d in (cp_x_b, cp_wg, cp_wu, cp_wd, cp_wo, cp_wmod_b):
        d.start()

    NW = 3 * D // 128

    def wqkv_t(i):
        for k in range(NW // 2):
            tmp_pad[dtile(i * (NW // 2) + k), :] = wqkv_in[:, dtile(i * (NW // 2) + k)].T

    loop(2, wqkv_t)
    tmp_pad[NW * 128:3 * D, :] = wqkv_in[:, NW * 128:3 * D].T

    def wqkv_pad(i):
        stages = [pad_stages(tmp_pad, 3 * i + k, wqkvT, k) for k in range(3)]
        for step in range(2):
            for k in range(3):
                stages[k][step]()

    loop(HP // 128, wqkv_pad)

    c = c_ref[...].astype(F32)
    sig_c = 1.0 / (1.0 + jnp.exp(-c))
    sc = c * sig_c
    row16 = jax.lax.broadcasted_iota(jnp.int32, (16, D), 0)
    hi, mid, lo = _split3(sc)
    sc3 = jnp.where(row16 == 0, hi, jnp.where(row16 == 1, mid, jnp.where(row16 == 2, lo, 0.0))).astype(BF16)

    def mod_tile(i):
        mod3 = _dot(sc3, wmod_in[:, dtile(i)])
        mod = mod3[0:1] + mod3[1:2] + mod3[2:3]
        modc[dtile(i), :] = jnp.broadcast_to(mod, (128, 128)).T

    def mcol(i):
        return modc[i * D:(i + 1) * D, :]

    SA, CA, GA, SB, CB, GB = range(6)
    NA, NM = MA // 128, 6 * D // 128

    cp_wmod_a.wait()
    for i in range(NA):
        mod_tile(i)

    QC = 256
    rowq = jax.lax.broadcasted_iota(jnp.int32, (QC, 128), 0) % DP
    is_one = jnp.logical_and(rowq >= DH, rowq < DH + 3)

    def ln1_stages(t):
        def finish(xh, rs):
            xh1[t] = xh
            st1[t] = jnp.broadcast_to(rs, (8, 128))
            h1T[t] = (xh * (1.0 + mcol(CA)) + mcol(SA)).astype(BF16)

        return _layernorm_stages(lambda: x_in[:, dtile(t)].astype(F32), finish)

    def qkv_chunk(t, ci, h1):
        r = _dot(wqkvT[ci * QC:(ci + 1) * QC, :], h1)
        part, sub = divmod(ci, HP // QC)
        rows = slice(sub * QC, (sub + 1) * QC)
        if part == 0:
            r = r * (SCALE * LOG2E)
            qT[t, rows, :] = r.astype(BF16)
        if part < 2:
            n2 = jnp.sum((r * r).reshape(QC // DP, DP, 128), axis=1)
            nrm[2 * part + sub] = jnp.maximum(nrm[2 * part + sub], n2)
        if part > 0:
            rb = jnp.where(is_one, 1.0, r).astype(BF16)
            dst_t, dst_tm = (kT, k_tm) if part == 1 else (vT, v_tm)
            dst_t[t, rows, :] = rb
            for gi in range(QC // 128):
                dst_tm[sub * (QC // 128) + gi, dtile(t), :] = rb[gi * 128:(gi + 1) * 128, :].T

    def qkv_tile(t, side_jobs):
        h1 = h1T[t]
        main = [lambda ci=ci: qkv_chunk(t, ci, h1) for ci in (4, 5, 2, 3, 0, 1)]
        ln = ln1_stages(jnp.minimum(t + 1, NTT - 1))
        _interleave(main, ln + side_jobs)

    def transpose_into(dst, didx, src, sidx):
        def job():
            dst[didx] = src[sidx].T
        return job

    def qkv_a(t):
        qkv_tile(t, [])

    def qkv_b(t):
        i = t - TA
        jobs = []
        for k in range(2):
            f = jnp.minimum(2 * i + k, NF - 1)
            for dst, src in ((wgT, wg_in), (wuT, wu_in), (wdN, wd_in)):
                jobs.append(transpose_into(dst, (dtile(f), slice(None)), src, (slice(None), dtile(f))))
            jobs.append(lambda k=k: mod_tile(NA + jnp.minimum(2 * i + k, NM - NA - 1)))
        g = jnp.minimum(i, HP // 128 - 1)
        wo_pad = pad_stages(wo_in, g, woP)
        wo_t = transpose_into(woT, (slice(None), dtile(g)), woP, (dtile(g), slice(None)))
        qkv_tile(t, [jobs[3], wo_pad[0], jobs[7], wo_pad[1], jobs[0], jobs[1], wo_t, jobs[2],
                     jobs[4], jobs[5], jobs[6]])

    cp_x_0.wait()
    for stage in ln1_stages(0):
        stage()
    cp_x_a.wait()
    loop(TA, qkv_a)
    cp_dy.start()
    for d in (cp_x_b, cp_wg, cp_wu, cp_wd, cp_wo, cp_wmod_b):
        d.wait()
    loop(NTT, qkv_b, start=TA)
    cp_dy.wait()

    qmax = jnp.max(nrm[0:2], axis=2, keepdims=True)
    kmax = jnp.max(nrm[2:4], axis=2, keepdims=True)
    bound2 = jnp.max(qmax * kmax)
    flag[0] = jnp.where(bound2 <= SAFE_BOUND * SAFE_BOUND, 0, 1).astype(jnp.int32)

    row16l = jax.lax.broadcasted_iota(jnp.int32, (16, 128), 0)

    def put3(base16, v):
        hi, mid, lo = _split3(v)
        return jnp.where(row16l == 12, -hi,
                         jnp.where(row16l == 13, -mid, jnp.where(row16l == 14, -lo, base16)))

    def block_body(b, carry):
        tq = [b * NQ + j for j in range(NQ)]
        tok = [pl.ds(pl.multiple_of(tq[j] * 128, 128), 128) for j in range(NQ)]
        lanes = [slice(j * 128, (j + 1) * 128) for j in range(NQ)]

        def carry_over(old):
            return jnp.where(b > 0, old, 0.0)

        for h in range(H):
            for j in range(NQ):
                wq[h, j, (h % 4) * DP:(h % 4 + 1) * DP, :] = qT[tq[j], hrows[h], :]

        @pl.when(flag[0] != 0)
        def _():
            def max_body(h, c2):
                dst = pl.multiple_of((h % 4) * DP + 16, 16)
                for j in range(NQ):
                    def key_tile(t, m):
                        s = _dot(k_tm[h // 4, dtile(t), :], wq[h, j])
                        return jnp.maximum(m, jnp.max(s, axis=0, keepdims=True))

                    m = jax.lax.fori_loop(0, NTT, key_tile, jnp.full((1, 128), -jnp.inf, F32))
                    old = wq[h, j, pl.ds(dst, 16), :].astype(F32)
                    wq[h, j, pl.ds(dst, 16), :] = put3(old, m).astype(BF16)
                return c2

            jax.lax.fori_loop(0, H, max_body, 0)

        for j in range(NQ):
            dffn[:, lanes[j]] = (dy_in[:, tok[j]].astype(F32) * mcol(GB)).astype(BF16)

        seq = [(hh, gi) for hh in range(HL) for gi in range(NG)]

        def head_rows(h):
            return pl.ds(pl.multiple_of(h * DP, DP), DP)

        fcol = [slice(f * FC, (f + 1) * FC) for f in range(NF)]

        def ffn_da(f):
            rows = fcol[f] if isinstance(f, int) else dtile(f)
            da_s[f % NDA] = _dot(wdN[rows, :], dffn[...])

        def fwd_body(it, c2):
            def s_group(hh, gi):
                h = it * HL + hh
                for j in range(NQ):
                    for t in range(gi * KG, (gi + 1) * KG):
                        s = _dot(k_tm[h // 4, tile[t], :], wq[h, j])
                        p_s[h, j, tile[t], :] = jnp.exp2(s).astype(BF16)

            def pv_group(hh, gi, acc):
                h = it * HL + hh
                for t in range(gi * KG, (gi + 1) * KG):
                    for j in range(NQ):
                        r = _dot(vT[t, head_rows(h), :], p_s[h, j, tile[t], :])
                        acc[j] = r if acc[j] is None else acc[j] + r

            def finish_head(hh, acc):
                h = it * HL + hh
                for j in range(NQ):
                    rl = 1.0 / acc[j][DH:DH + 1, :]
                    o = acc[j] * rl
                    ot[head_rows(h), lanes[j]] = o
                    otb[head_rows(h), lanes[j]] = o.astype(BF16)
                    rl_s[h, j] = jnp.broadcast_to(rl, (8, 128))

            def wo_part(gg):
                g0 = pl.multiple_of((it * (HL // 4) + gg) * 128, 128)
                for half in range(2):
                    rows = slice(half * (D // 2), (half + 1) * (D // 2))
                    r = _dot(woT[rows, pl.ds(g0, 128)], otb[pl.ds(g0, 128), :])
                    if gg == 0:
                        attn[rows, :] = jnp.where(it > 0, attn[rows, :], 0.0) + r
                    else:
                        attn[rows, :] += r

            acc = None
            wo_due = []
            for n in range(len(seq) + LAGF):
                if n < len(seq):
                    s_group(*seq[n])
                if n >= LAGF:
                    hh, gi = seq[n - LAGF]
                    if gi == 0:
                        acc = [None] * NQ
                    pv_group(hh, gi, acc)
                    if n == len(seq) + LAGF - 1:
                        ffn_da(it)
                    if gi == NG - 1:
                        finish_head(hh, acc)
                        if hh % 4 == 3:
                            wo_due.append((n + 2, hh // 4))
                if wo_due and (wo_due[0][0] <= n or n == len(seq) + LAGF - 1):
                    wo_part(wo_due.pop(0)[1])
            return c2

        jax.lax.fori_loop(0, H // HL, fwd_body, 0)

        def ffn_gu(f):
            g = _dot(wgT[fcol[f], :], h2[...])
            u = _dot(wuT[fcol[f], :], h2[...])
            da = da_s[f % NDA]
            sg = 0.5 * jnp.tanh(0.5 * g) + 0.5
            si = g * sg
            act_s[f % 3] = (si * u).astype(BF16)
            dgu_s[f % 3, 0:FC, :] = (da * u * (sg + si * (1.0 - sg))).astype(BF16)
            dgu_s[f % 3, FC:2 * FC, :] = (da * si).astype(BF16)

        def ffn_out(f):
            r = _dot(wd_in[:, fcol[f]], act_s[f % 3])
            d = _dot(wg_in[:, fcol[f]], dgu_s[f % 3, 0:FC, :]) + _dot(wu_in[:, fcol[f]], dgu_s[f % 3, FC:2 * FC, :])
            if f == 0:
                ffn[...] = r
                dh2[...] = d
            else:
                ffn[...] += r
                dh2[...] += d

        def dw_update(acc_ref, st_ref, f, r):
            new = carry_over(acc_ref[:, fcol[f]]) + r
            acc_ref[:, fcol[f]] = new
            st_ref[:, fcol[f]] = new.astype(BF16)

        def ffn_dw_gu(f, z=None):
            lh = h2[...] if z is None else _after(h2[...], z)
            dgu = _dot_nt(lh, dgu_s[f % 3])
            dw_update(dwg_acc, dwg_st, f, dgu[:, 0:FC])
            dw_update(dwu_acc, dwu_st, f, dgu[:, FC:2 * FC])

        def ffn_dw_d(f, z=None):
            ld = dffn[...] if z is None else _after(dffn[...], z)
            dw_update(dwd_acc, dwd_st, f, _dot_nt(ld, act_s[f % 3]))

        def ffn_dw(f):
            ffn_dw_gu(f)
            ffn_dw_d(f)

        def ln2_stages(j):
            def residual():
                x1j = x_in[:, tok[j]].astype(F32) + mcol(GA) * attn[:, lanes[j]]
                x1[:, lanes[j]] = x1j
                return x1j

            def finish(xh, rs):
                xh2[:, lanes[j]] = xh
                st2[j] = jnp.broadcast_to(rs, (8, 128))
                h2[:, lanes[j]] = (xh * (1.0 + mcol(CB)) + mcol(SB)).astype(BF16)

            return _layernorm_stages(lambda: x1[:, lanes[j]], finish, first_load=residual)

        def ln2_fwd():
            ln = [ln2_stages(j) for j in range(NQ)]
            for k in range(3):
                ffn_da(k + H // HL)
                for j in range(NQ):
                    ln[j][k]()

        def ffn_step(f):
            ffn_gu(f)
            if f >= 1 and f + NDA - 1 < NF:
                ffn_da(f + NDA - 1)
            if f >= 1:
                ffn_out(f - 1)
            if f >= 2:
                ffn_dw(f - 2)

        ln2_fwd()
        for f in range(NF):
            ffn_step(f)
        ffn_out(NF - 1)

        z2 = _zero_after(dh2[0:1, :])
        row32 = jax.lax.broadcasted_iota(jnp.int32, (DP, 128), 0)
        dyt = [lambda j=j: dy_in[:, tok[j]].astype(F32) for j in range(NQ)]
        m12 = {}

        def ln2_bwd_a(j):
            dxh = dh2[:, lanes[j]] * (1.0 + mcol(CB))
            m12[j] = (jnp.mean(dxh, axis=0, keepdims=True),
                      jnp.mean(dxh * xh2[:, lanes[j]], axis=0, keepdims=True))

        def ln2_bwd_b(j):
            dxh = dh2[:, lanes[j]] * (1.0 + mcol(CB))
            dx1 = dyt[j]() + st2[j, 0:1, :] * (dxh - m12[j][0] - xh2[:, lanes[j]] * m12[j][1])
            dx1T[tq[j]] = dx1
            dattn[:, lanes[j]] = (dx1 * mcol(GA)).astype(BF16)

        def dmod_acc(i, term):
            tot = term(0)
            for j in range(1, NQ):
                tot = tot + term(j)
            dmodp[i * D:(i + 1) * D, :] += tot

        def block_out(j):
            out_st[b % 2, :, lanes[j]] = (x1[:, lanes[j]] + mcol(GB) * ffn[:, lanes[j]]).astype(BF16)

        def do_part(g):
            do_s[g * 128:(g + 1) * 128, :] = _dot(woP[g * 128:(g + 1) * 128, :], dattn[...])

        def prep_head(h):
            r0 = pl.multiple_of((h % 4) * DP, DP)
            for j in range(NQ):
                do = do_s[head_rows(h), lanes[j]]
                rl = rl_s[h, j, 0:1, :]
                delta = jnp.sum(do * ot[head_rows(h), lanes[j]], axis=0, keepdims=True) * rl
                hi, mid, lo = _split3(delta)
                dov = jnp.where(row32 == DH, -hi,
                                jnp.where(row32 == DH + 1, -mid,
                                          jnp.where(row32 == DH + 2, -lo, do * rl))).astype(BF16)
                dob[j, head_rows(h), :] = dov
                wdo[h, j, pl.ds(r0, DP), :] = dov

        ffn_dw_gu(NF - 2, z2)
        for j in range(NQ):
            ln2_bwd_a(j)
        ffn_dw_d(NF - 2, z2)
        for j in range(NQ):
            ln2_bwd_b(j)
        ffn_dw_gu(NF - 1, z2)
        dmod_acc(SB, lambda j: dh2[:, lanes[j]])
        do_part(0)
        dmod_acc(CB, lambda j: dh2[:, lanes[j]] * xh2[:, lanes[j]])
        ffn_dw_d(NF - 1, z2)
        prep_head(0)
        dmod_acc(GB, lambda j: dyt[j]() * ffn[:, lanes[j]])
        dmod_acc(GA, lambda j: dx1T[tq[j]] * attn[:, lanes[j]])
        do_part(1)
        block_out(0)
        do_part(2)
        block_out(1)
        do_part(3)

        def bwd_body(it, c2):
            def dp_group(hh, gi):
                h = it * HL + hh
                for t in range(gi * KG, (gi + 1) * KG):
                    vc = v_tm[h // 4, tile[t], :]
                    for j in range(NQ):
                        dp = _dot(vc, wdo[h, j])
                        ds_s[hh % 2, j, tile[t], :] = (p_s[h, j, tile[t], :].astype(F32) * dp).astype(BF16)

            def g_group(hh, gi, acc):
                h = it * HL + hh
                ts = list(range(gi * KG, (gi + 1) * KG))
                dk, dv = {}, {}
                for t in ts:
                    for j in range(NQ):
                        r = _dot_nt(dob[j, head_rows(h), :], p_s[h, j, tile[t], :])
                        dv[t] = r if t not in dv else dv[t] + r
                for t in ts:
                    for j in range(NQ):
                        r = _dot_nt(qT[tq[j], head_rows(h), :], ds_s[hh % 2, j, tile[t], :])
                        dk[t] = r if t not in dk else dk[t] + r
                for t in ts:
                    for j in range(NQ):
                        r = _dot(kT[t, head_rows(h), :], ds_s[hh % 2, j, tile[t], :])
                        acc[j] = r if acc[j] is None else acc[j] + r
                for t in ts:
                    dkT[t, head_rows(h), :] = carry_over(dkT[t, head_rows(h), :]) + dk[t]
                    dvT[t, head_rows(h), :] = carry_over(dvT[t, head_rows(h), :]) + dv[t]

            def dwo_part():
                cols = pl.ds(pl.multiple_of(it * (HL * DP), HL * DP), HL * DP)
                dwo_acc[:, cols] = carry_over(dwo_acc[:, cols]) + _dot_nt(dattn[...], otb[cols, :])

            acc = None
            for n in range(len(seq) + LAGB):
                if n < len(seq):
                    hh, gi = seq[n]
                    if gi == NG - 2:
                        prep_head(jnp.minimum(it * HL + hh + 1, H - 1))
                    dp_group(hh, gi)
                if n == len(seq):
                    dwo_part()
                if n >= LAGB:
                    hh, gi = seq[n - LAGB]
                    if gi == 0:
                        acc = [None] * NQ
                    g_group(hh, gi, acc)
                    if gi == NG - 1:
                        for j in range(NQ):
                            dqT[tq[j], head_rows(it * HL + hh), :] = (acc[j] * SCALE).astype(BF16)
            return c2

        jax.lax.fori_loop(0, H // HL, bwd_body, 0)

        pltpu.make_async_copy(out_st.at[b % 2], out_hbm.at[:, pl.ds(pl.multiple_of(b * BQ, BQ), BQ)],
                              sems.at[10 + b % 2]).start()

        @pl.when(b > 0)
        def _():
            pltpu.make_async_copy(out_st.at[(b - 1) % 2],
                                  out_hbm.at[:, pl.ds(pl.multiple_of((b - 1) * BQ, BQ), BQ)],
                                  sems.at[10 + (b - 1) % 2]).wait()
        return carry

    jax.lax.fori_loop(0, NB, block_body, 0)
    pltpu.make_async_copy(out_st.at[(NB - 1) % 2], out_hbm.at[:, pl.ds((NB - 1) * BQ, BQ)],
                          sems.at[10 + (NB - 1) % 2]).wait()

    sccol = jnp.broadcast_to(sc, (128, D)).T
    row16t = jax.lax.broadcasted_iota(jnp.int32, (16, 128), 0)

    def dmod_stages(i, slot, box):
        st = {}

        def s1():
            st["dm"] = jnp.sum(dmodp[dtile(i), :].T, axis=0, keepdims=True)

        def s2():
            dwmod_st[slot] = (sccol * st["dm"]).astype(BF16)

        def s3():
            hi, mid, lo = _split3(st["dm"])
            dm3 = jnp.where(row16t == 0, hi, jnp.where(row16t == 1, mid, jnp.where(row16t == 2, lo, 0.0)))
            box.append(_dot_nt(dm3.astype(BF16), wmod_in[:, dtile(i)]))

        return [s1, s2, s3]

    def unpad_stages(get_block, g, dst, k=0):
        def s1():
            s128u[k] = get_block()

        def s2():
            for hh in range(4):
                s112[k, DH * hh:DH * hh + DH, :] = s128u[k, DP * hh:DP * hh + DH, :]
            dst[pl.ds(pl.multiple_of(g * GD, 16), GD), :] = s112[k]

        return [s1, s2]

    def ln1_bwd_stages(t, slot):
        st = {}

        def rows_of(base, hi):
            return slice(base * D + halves[hi].start, base * D + halves[hi].stop)

        def dsa(hi):
            dmodp[rows_of(SA, hi), :] += dh_s[slot, halves[hi], :]

        def dca(hi):
            dmodp[rows_of(CA, hi), :] += dh_s[slot, halves[hi], :] * xh1[t, halves[hi], :]

        def dxh(hi):
            return dh_s[slot, halves[hi], :] * (1.0 + modc[rows_of(CA, hi), :])

        def stats(hi):
            d = dxh(hi)
            s1 = jnp.sum(d, axis=0, keepdims=True)
            s2 = jnp.sum(d * xh1[t, halves[hi], :], axis=0, keepdims=True)
            st[hi] = (s1, s2)

        def out(hi):
            m1 = (st[0][0] + st[1][0]) * (1.0 / D)
            m2 = (st[0][1] + st[1][1]) * (1.0 / D)
            dx = dx1T[t, halves[hi], :] + st1[t, 0:1, :] * (dxh(hi) - m1 - xh1[t, halves[hi], :] * m2)
            dx_st[halves[hi], dtile(t)] = dx.astype(BF16)

        return [lambda fn=fn, hi=hi: fn(hi) for fn in (dsa, dca, stats, out) for hi in range(2)]

    def conv_stages(t):
        def drop_pads(part, src):
            for h in range(H):
                dqkvU[t, part * D + DH * h:part * D + DH * (h + 1), :] = src(slice(DP * h, DP * h + DH))

        def cq():
            drop_pads(0, lambda rows: dqT[t, rows, :])
            dqkvU[t, 3 * D:NWC * 128, :] = jnp.zeros((NWC * 128 - 3 * D, 128), BF16)

        def ck1():
            cv_s[0] = (dkT[t] * LN2).astype(BF16)

        def ck2():
            drop_pads(1, lambda rows: cv_s[0, rows, :])

        def cv1():
            cv_s[1] = dvT[t].astype(BF16)

        def cv2():
            drop_pads(2, lambda rows: cv_s[1, rows, :])

        return [cq, ck1, ck2, cv1, cv2]

    cp_dwg = cp(dwg_st, dwg_hbm, 0)
    cp_dwu = cp(dwu_st, dwu_hbm, 1)
    cp_dwd = cp(dwd_st, dwd_hbm, 2)
    cp_dwo = cp(dwo_st.at[0:D, :], dwo_hbm, 3)
    cp_dx = cp(dx_st, dx_hbm, 4)

    for d in (cp_dwg, cp_dwu, cp_dwd):
        d.start()

    kparts = [slice(0, 512), slice(512, 1024), slice(1024, 3 * D)]

    def dx_tile(t):
        acc = {}

        def mm(src, hi):
            r = _dot(wqkv_in[halves[hi], kparts[src]], dqkvU[t, kparts[src], :])
            acc[hi] = r if src == 0 else acc[hi] + r
            if src == 2:
                dh_s[t % 2, halves[hi], :] = acc[hi]

        ln = ln1_bwd_stages(jnp.maximum(t - 1, 0), (t + 1) % 2)
        cq, ck1, ck2, cv1, cv2 = conv_stages(jnp.minimum(t + 1, NTT - 1))
        main = [lambda src=src, hi=hi: mm(src, hi) for hi in range(2) for src in range(3)]
        side = [ck1, cv1, ln[4], ln[5], ck2, ln[0], ln[6], cv2, ln[1], ln[7], cq, ln[2], ln[3]]
        _interleave(main, side)

    dh_s[1] = jnp.zeros((D, 128), F32)
    for stage in conv_stages(0):
        stage()
    loop(NTT, dx_tile)
    for stage in ln1_bwd_stages(NTT - 1, (NTT - 1) % 2):
        stage()

    cp_dx.start()

    def cp_dwqkv_tile(n, cols):
        return cp(dwqkv_st.at[n], dwqkv_hbm.at[:, cols], 8)

    def cp_dwmod_tile(i, cols):
        return cp(dwmod_st.at[i], dwmod_hbm.at[:, cols], 6)

    def dwqkv_body(n, dsc3):
        accs = [None, None]

        def mm(hi, t):
            def job():
                r = _dot_nt(h1T[t, halves[hi], :], dqkvU[t, dtile(n), :])
                accs[hi] = r if accs[hi] is None else accs[hi] + r
                if t == NTT - 1:
                    dwqkv_st[n, halves[hi], :] = accs[hi].astype(BF16)
            return job

        box = []
        mods = [2 * n, 2 * n + 1]
        dm = [dmod_stages(jnp.minimum(i, NM - 1), jnp.minimum(i, NM), box) for i in mods]
        g = jnp.minimum(n, HP // 128 - 1)
        wo = unpad_stages(lambda: dwo_acc[:, dtile(g)].astype(BF16).T, jnp.minimum(n, HP // 128), dwo_st, 1)
        _interleave([mm(hi, t) for hi in range(2) for t in range(NTT)],
                    [dm[0][0], wo[0], dm[1][0], dm[0][1], wo[1], dm[0][2], dm[1][1], dm[1][2]], first=1)

        @pl.when(n < NWC - 1)
        def _():
            cp_dwqkv_tile(n, dtile(n)).start()

        cp_dwmod_tile(mods[0], dtile(mods[0])).start()

        @pl.when(mods[1] < NM)
        def _():
            cp_dwmod_tile(mods[1], dtile(mods[1])).start()

        @pl.when(n == HP // 128)
        def _():
            cp_dwo.start()

        return dsc3 + box[0] + jnp.where(mods[1] < NM, box[1], 0.0)

    assert 2 * NWC - 1 == NM
    dsc3 = jax.lax.fori_loop(0, NWC, dwqkv_body, jnp.zeros((16, D), F32))
    w_last = 3 * D - (NWC - 1) * 128
    dwqkv_last[...] = dwqkv_st[NWC - 1, :, 0:w_last]
    cp_dwqkv_last = cp(dwqkv_last, dwqkv_hbm.at[:, (NWC - 1) * 128:3 * D], 9)
    cp_dwqkv_last.start()
    dsc = dsc3[0:1] + dsc3[1:2] + dsc3[2:3]
    dc_ref[...] = (dsc * (sig_c * (1.0 + c * (1.0 - sig_c)))).astype(BF16)
    cp_dwqkv = [cp_dwqkv_tile(k, tile[k]) for k in range(NWC - 1)] + [cp_dwqkv_last]
    cp_dwmod = [cp_dwmod_tile(i, tile[i]) for i in range(NM)]

    for d in (cp_dwg, cp_dwu, cp_dwd, cp_dwo, cp_dx, *cp_dwmod, *cp_dwqkv):
        d.wait()


def _scratch():
    v = pltpu.VMEM
    return [
        v((D, T), BF16), v((D, T), BF16), v((D, 3 * D), BF16), v((D, D), BF16),
        v((D, F), BF16), v((D, F), BF16), v((D, F), BF16), v((D, 6 * D), BF16),
        v((3 * HP, D), BF16), v((D, HP), BF16), v((HP, D), BF16),
        v((F, D), BF16), v((F, D), BF16), v((F, D), BF16), v((3 * D, D), BF16),
        v((3, 4 * DH, D), BF16), v((3, 128, D), BF16), v((2, 128, D), BF16),
        v((6 * D, 128), F32), v((6 * D, 128), F32),
        v((NTT, D, 128), F32), v((NTT, 8, 128), F32), v((NTT, D, 128), BF16),
        v((NTT, HP, 128), BF16), v((NTT, HP, 128), BF16), v((NTT, HP, 128), BF16),
        v((4, T, 128), BF16), v((4, T, 128), BF16),
        v((NTT, HP, 128), BF16), v((NTT, HP, 128), F32), v((NTT, HP, 128), F32),
        v((NTT, NWC * 128, 128), BF16), v((2, HP, 128), BF16),
        v((NTT, D, 128), F32), v((4, 8, 128), F32),
        v((H, NQ, 128, 128), BF16), v((H, NQ, 128, 128), BF16),
        v((H, NQ, T, 128), BF16), v((2, NQ, T, 128), BF16),
        v((HP, BQ), F32), v((HP, BQ), BF16), v((H, NQ, 8, 128), F32),
        v((D, BQ), F32), v((D, BQ), F32), v((D, BQ), F32), v((NQ, 8, 128), F32),
        v((D, BQ), BF16), v((D, BQ), BF16),
        v((D, BQ), F32), v((D, BQ), F32),
        v((NDA, FC, BQ), F32), v((3, FC, BQ), BF16), v((3, 2 * FC, BQ), BF16),
        v((D, BQ), BF16), v((HP, BQ), F32), v((NQ, HP, 128), BF16), v((2, D, 128), F32),
        v((D, F), F32), v((D, F), F32), v((D, F), F32), v((D, HP), F32),
        v((2, D, BQ), BF16), v((D, T), BF16), v((D, F), BF16), v((D, F), BF16), v((D, F), BF16),
        v((D + 4 * DH, D), BF16), v((NWC, D, 128), BF16), v((D, 3 * D - (NWC - 1) * 128), BF16),
        v((6 * D // 128 + 1, D, 128), BF16),
        pltpu.SMEM((1,), jnp.int32),
        pltpu.SemaphoreType.DMA((13,)),
    ]


@jax.jit
def pallas_adaLN_cond__softmax_full_mha__swiglu_ffn__prompt_kernel(
    A_x: jax.Array,
    A_wqkv: jax.Array,
    A_wo: jax.Array,
    B_x: jax.Array,
    B_w_gate: jax.Array,
    B_w_up: jax.Array,
    B_w_down: jax.Array,
    c: jax.Array,
    w_mod: jax.Array,
    grad_out: jax.Array,
):
    del B_x
    sds = jax.ShapeDtypeStruct
    hbm = pl.BlockSpec(memory_space=pl.ANY)
    vmem = pl.BlockSpec(memory_space=pltpu.VMEM)
    outs = pl.pallas_call(
        _kernel,
        out_shape=(
            sds((D, T), BF16), sds((D, T), BF16), sds((D, 3 * D), BF16), sds((D, D), BF16),
            sds((D, F), BF16), sds((D, F), BF16), sds((D, F), BF16), sds((1, D), BF16),
            sds((D, 6 * D), BF16),
        ),
        in_specs=[hbm] * 8 + [vmem],
        out_specs=(hbm,) * 7 + (vmem, hbm),
        scratch_shapes=_scratch(),
        compiler_params=pltpu.CompilerParams(vmem_limit_bytes=120 * 1024 * 1024),
        name="adaln_block_fwd_bwd",
    )(A_x.reshape(T, D).T, A_wqkv, A_wo, B_w_gate, B_w_up, B_w_down.T, w_mod,
      grad_out.reshape(T, D).T, c)
    out, dx, dwqkv, dwo, dwg, dwu, dwd, dc, dwmod = outs
    return (out.T.reshape(1, T, D), dx.T.reshape(1, T, D), dwqkv, dwo, dwg, dwu, dwd.T, dc, dwmod)
```
